```python
import jax
import jax.numpy as jnp

def _softmax(x, axis=-1):
    return jax.nn.softmax(x, axis=axis)
def _gelu(x):
    return jax.nn.gelu(x, approximate=True)
def _silu(x):
    return jax.nn.silu(x)
def _sigmoid(x):
    return jax.nn.sigmoid(x)
def _layernorm(x, axis=-1, eps=1e-5):
    m = jnp.mean(x, axis=axis, keepdims=True)
    v = jnp.var(x, axis=axis, keepdims=True)
    return (x - m) / jnp.sqrt(v + eps)
def _scatter_add(tgt, idx, src, axis=0):
    return tgt.at[idx].add(src)
def _segment_sum(src, seg, n):
    return jax.ops.segment_sum(src, seg, n)
class _Rng:
    def __init__(self, key):
        self._k = key
    def _next(self):
        self._k, sub = jax.random.split(self._k)
        return sub
    def normal(self, shape):
        return jax.random.normal(self._next(), shape, dtype=jnp.bfloat16)
    def randint(self, lo, hi, shape):
        return jax.random.randint(self._next(), shape, lo, hi, dtype=jnp.int32)
    def uniform(self, shape, lo=0.0, hi=1.0):
        return jax.random.uniform(self._next(), shape, jnp.bfloat16, lo, hi)
    def permutation(self, n):
        return jax.random.permutation(self._next(), n)


kernel_name = 'standalone__fft_conv__vision'

def setup_inputs():
    _rng = _Rng(jax.random.key(int.from_bytes(__import__("os").urandom(4), "little")))
    _w = (lambda a: (lambda t: t.astype(jnp.bfloat16) if jnp.issubdtype(t.dtype, jnp.floating) else t)(jnp.asarray(a)))
    H = W = 224
    C = 96
    K = 7
    return {
        "x": _w((lambda *s: _rng.normal(s) * 0.05)(1, H, W, C)),
        "w": _w((lambda *s: _rng.normal(s) * 0.05)(K, K, C, C)),
    }

def reference(x, w):
    B, H, W, C = x.shape
    K = w.shape[0]
    wp = jnp.pad(w, ((0, H - K), (0, W - K), (0, 0), (0, 0)))
    Xf = (lambda x, axes=(-2,-1): jnp.fft.rfft2(x.astype(jnp.float32), axes=axes))(x, axes=(1, 2))
    Wf = (lambda x, axes=(-2,-1): jnp.fft.rfft2(x.astype(jnp.float32), axes=axes))(wp, axes=(0, 1))
    Yf = jnp.einsum('bhwi,hwio->bhwo', Xf, Wf)
    y = (lambda x, s, axes=(-2,-1): jnp.fft.irfft2(x, s=s, axes=axes).astype(jnp.bfloat16))(Yf, (H, W), axes=(1, 2))
    return y
```

```python
import math
import jax
import jax.numpy as jnp
import numpy as np
import jax.experimental.pallas as pl
import jax.experimental.pallas.tpu as pltpu


class V:
    __slots__ = ("s", "a")
    def __init__(self, a, s=1): self.a = a; self.s = s
    def neg(self): return V(self.a, -self.s)

class Ctx:
    def __init__(self): self.nadd = 0; self.nmul = 0
    def add(self, x, y):
        if x.a is None: return y
        if y.a is None: return x
        self.nadd += 1
        if x.s == y.s: return V(x.a + y.a, x.s)
        if x.s > 0: return V(x.a - y.a, 1)
        return V(y.a - x.a, 1)
    def sub(self, x, y): return self.add(x, y.neg())
    def mul(self, x, c):
        if x.a is None or c == 0: return V(None)
        if c == 1: return x
        if c == -1: return x.neg()
        self.nmul += 1
        return V(x.a * np.float32(c * x.s), 1)
    def cmul(self, xr, xi, c, s):
        if abs(abs(c) - abs(s)) < 1e-12 and abs(c) > 1e-12:
            if (c > 0) == (s > 0):
                return self.mul(self.sub(xr, xi), c), self.mul(self.add(xr, xi), c)
            else:
                return self.mul(self.add(xr, xi), c), self.mul(self.sub(xi, xr), c)
        return (self.sub(self.mul(xr, c), self.mul(xi, s)), self.add(self.mul(xr, s), self.mul(xi, c)))

def _tw(k, n):
    c, s = math.cos(2*math.pi*k/n), -math.sin(2*math.pi*k/n)
    if abs(c) < 1e-12: c = 0.0
    if abs(s) < 1e-12: s = 0.0
    return c, s

def rfft(ctx, x):
    n = len(x)
    if n == 1:
        return [x[0]], [V(None)]
    if n == 2:
        return [ctx.add(x[0], x[1]), ctx.sub(x[0], x[1])], [V(None), V(None)]
    er, ei = rfft(ctx, x[0::2])
    orr, oi = rfft(ctx, x[1::2])
    h = n // 2; q = n // 4
    re = [None]*(h+1); im = [None]*(h+1)
    re[0] = ctx.add(er[0], orr[0]); re[h] = ctx.sub(er[0], orr[0]); im[0] = V(None); im[h] = V(None)
    re[q] = er[q]; im[q] = orr[q].neg()
    for k in range(1, q):
        c, s = _tw(k, n)
        tr, ti = ctx.cmul(orr[k], oi[k], c, s)
        re[k] = ctx.add(er[k], tr); im[k] = ctx.add(ei[k], ti)
        re[h-k] = ctx.sub(er[k], tr); im[h-k] = ctx.sub(ti, ei[k])
    return re, im

def irfft(ctx, re, im):
    h = len(re) - 1; n = 2*h
    if n == 0 or h == 0:
        return [re[0]]
    if n == 2:
        return [ctx.add(re[0], re[1]), ctx.sub(re[0], re[1])]
    q = n // 4
    er = [None]*(q+1); ei = [None]*(q+1); orr = [None]*(q+1); oi = [None]*(q+1)
    er[0] = ctx.add(re[0], re[h]); orr[0] = ctx.sub(re[0], re[h]); ei[0] = V(None); oi[0] = V(None)
    er[q] = re[q]; orr[q] = im[q].neg(); ei[q] = V(None); oi[q] = V(None)
    for k in range(1, q):
        er[k] = ctx.add(re[k], re[h-k]); ei[k] = ctx.sub(im[k], im[h-k])
        tr = ctx.sub(re[k], re[h-k]); ti = ctx.add(im[k], im[h-k])
        c, s = _tw(k, n)
        orr[k], oi[k] = ctx.cmul(tr, ti, c, -s)
    xe = irfft(ctx, er, ei); xo = irfft(ctx, orr, oi)
    out = [None]*n
    out[0::2] = xe; out[1::2] = xo
    return out


H=W=224; C=96; K=7
T=64; HOP=56; NT=H//HOP
KK=K*2*C
WP=256

def val(v):
    return v.a if v.s > 0 else -v.a

def coef_table():
    tab = np.zeros((32*8, 384), np.float32)
    ri = (np.arange(384)//96) % 2
    for p in range(32):
        th = 2*math.pi*p/T
        for d in range(4):
            if p == 0:
                ct = np.where(ri==0, 1.0/T, 0.0)
                cb = np.where(ri==0, 0.0, math.cos(math.pi*d)/T)
            else:
                ct = np.where(ri==0, math.cos(th*d), math.sin(th*d))*2/T
                cb = np.where(ri==0, -math.sin(th*d), math.cos(th*d))*2/T
            tab[p*8+d] = ct; tab[p*8+4+d] = cb
    return tab

def kern(xm_ref, xh_ref, w_ref, ct_ref, o_ref, a_ref, u_ref, xe_ref, xf_ref):
    t = pl.program_id(0)

    @pl.when(t == 0)
    def _():
        ii = jax.lax.broadcasted_iota(jnp.int32, (C, C), 0) == jax.lax.broadcasted_iota(jnp.int32, (C, C), 1)
        eye = ii.astype(jnp.bfloat16)
        def wT(a):
            r = jnp.concatenate([w_ref[a, b] for b in range(K) for _ in range(2)], axis=0)
            return jax.lax.dot_general(eye, r, (((1,), (1,)), ((), ())), preferred_element_type=jnp.float32)
        lane = jax.lax.broadcasted_iota(jnp.int32, (C, KK), 1)
        ri0 = ((lane // C) % 2) == 0
        w3 = wT(3)
        u_ref[0] = jnp.where(ri0, w3, 0.0)
        u_ref[4] = jnp.where(ri0, 0.0, w3)
        for d in range(1, 4):
            wp = wT(3+d); wm = wT(3-d)
            s = wp + wm; tt = wp - wm
            u_ref[d] = jnp.where(ri0, s, tt)
            u_ref[4+d] = jnp.where(ri0, tt, s)
        def gen(p, c):
            for tb in range(2):
                acc = None
                for d in range(4):
                    cv = ct_ref[pl.ds(p*8 + tb*4 + d, 1), :]
                    cv = jnp.concatenate([cv]*4, axis=1)[:, :KK]
                    term = u_ref[tb*4+d] * cv
                    acc = term if acc is None else acc + term
                a_ref[p, tb*C:(tb+1)*C, :] = acc.astype(jnp.bfloat16)
            return c
        jax.lax.fori_loop(0, 32, gen, 0)

    def stage(row):
        xp = jnp.concatenate([row, jnp.zeros((C, WP-W), jnp.bfloat16)], axis=1)
        v = pltpu.bitcast(xp, jnp.uint32)
        v0 = v[:, :128]; v1 = v[:, 128:]
        r0 = pltpu.roll(v0, 6, 1); r1 = pltpu.roll(v1, 6, 1); r2 = pltpu.roll(v1, 38, 1)
        lane = jax.lax.broadcasted_iota(jnp.int32, v0.shape, 1)
        e0 = jnp.where(lane < 6, r2, r0)
        e1 = jnp.where(lane < 6, r0, r1)
        e = jnp.concatenate([e0, e1], axis=1)
        return pltpu.bitcast(e, jnp.bfloat16).astype(jnp.float32)
    for n in range(6):
        xe_ref[n] = stage(xh_ref[0, 2+n])
    def sbody(n, c):
        xe_ref[6+n] = stage(xm_ref[0, n])
        return c
    jax.lax.fori_loop(0, HOP, sbody, 0)

    def fbody(j, c):
        r = pl.multiple_of((j // 2) * 8, 8); cc = pl.multiple_of((j % 2) * 128, 128)
        ctx = Ctx()
        xs = [V(xe_ref[n, pl.ds(r, 8), pl.ds(cc, 128)]) for n in range(T-2)] + [V(None), V(None)]
        re, im = rfft(ctx, xs)
        xf_ref[0, pl.ds(r, 8), pl.ds(cc, 128)] = val(re[0])
        xf_ref[1, pl.ds(r, 8), pl.ds(cc, 128)] = val(re[T//2])
        for k in range(1, T//2):
            xf_ref[2*k, pl.ds(r, 8), pl.ds(cc, 128)] = val(re[k])
            xf_ref[2*k+1, pl.ds(r, 8), pl.ds(cc, 128)] = val(im[k])
        return c
    jax.lax.fori_loop(0, 24, fbody, 0)

    def mbody(p, c):
        cols = {}
        for ri in range(2):
            v = pltpu.bitcast(xf_ref[2*p+ri].astype(jnp.bfloat16), jnp.uint32)
            v0 = v[:, :128]; v1 = v[:, 128:]
            lane = jax.lax.broadcasted_iota(jnp.int32, v0.shape, 1)
            for b in range(K):
                s = 6 - b
                if s == 0:
                    e = v
                else:
                    r0 = pltpu.roll(v0, 128 - s, 1); r1 = pltpu.roll(v1, 128 - s, 1)
                    e = jnp.concatenate([jnp.where(lane < 128 - s, r0, r1), r1], axis=1)
                cols[(b, ri)] = pltpu.bitcast(e, jnp.bfloat16)
        xcol = jnp.concatenate([cols[(b, ri)] for b in range(K) for ri in range(2)], axis=0)
        y = jnp.dot(a_ref[p], xcol, preferred_element_type=jnp.float32)
        xf_ref[2*p] = y[:C]
        xf_ref[2*p+1] = y[C:]
        return c
    jax.lax.fori_loop(0, 32, mbody, 0)

    def ibody(j, c):
        r = pl.multiple_of((j // 2) * 8, 8); cc = pl.multiple_of((j % 2) * 128, 128)
        ctx = Ctx()
        ld = lambda k: V(xf_ref[k, pl.ds(r, 8), pl.ds(cc, 128)])
        re = [ld(0)] + [ld(2*k) for k in range(1, T//2)] + [ld(1)]
        im = [V(None)] + [ld(2*k+1) for k in range(1, T//2)] + [V(None)]
        out = irfft(ctx, re, im)
        for n in range(3, 3+HOP):
            xe_ref[n-3, pl.ds(r, 8), pl.ds(cc, 128)] = val(out[n])
        return c
    jax.lax.fori_loop(0, 24, ibody, 0)

    def obody(n, c):
        o_ref[0, n] = xe_ref[n][:, :W].astype(jnp.bfloat16)
        return c
    jax.lax.fori_loop(0, HOP, obody, 0)

@jax.jit
def pallas_standalone__fft_conv__vision_kernel(x: jax.Array, w: jax.Array):
    xT = x.transpose(0, 1, 3, 2)
    ct = coef_table()
    yT = pl.pallas_call(
        kern,
        grid=(NT,),
        in_specs=[pl.BlockSpec((1, HOP, C, W), lambda t: (0, t, 0, 0)),
                  pl.BlockSpec((1, 8, C, W), lambda t: (0, (7*t + 27) % 28, 0, 0)),
                  pl.BlockSpec((K, K, C, C), lambda t: (0, 0, 0, 0)),
                  pl.BlockSpec((256, 384), lambda t: (0, 0))],
        out_specs=pl.BlockSpec((1, HOP, C, W), lambda t: (0, t, 0, 0)),
        out_shape=jax.ShapeDtypeStruct((1, H, C, W), jnp.bfloat16),
        scratch_shapes=[pltpu.VMEM((32, 2*C, KK), jnp.bfloat16),
                        pltpu.VMEM((8, C, KK), jnp.float32),
                        pltpu.VMEM((T-2, C, WP), jnp.float32),
                        pltpu.VMEM((T, C, WP), jnp.float32)],
        compiler_params=pltpu.CompilerParams(dimension_semantics=("arbitrary",), vmem_limit_bytes=100*1024*1024),
    )(xT, xT, w, ct)
    return yT.transpose(0, 1, 3, 2)
```

```python
import contextlib
import functools
import math

import jax
import jax.numpy as jnp
import numpy as np
import jax.experimental.pallas as pl
import jax.experimental.pallas.tpu as pltpu

class Cell:
    __slots__ = ("v", "fn")
    def __init__(self, fn=None): self.v = None; self.fn = fn
    def get(self):
        if self.v is None: self.v = self.fn()
        return self.v

class V:
    __slots__ = ("s", "a")
    def __init__(self, a, s=1): self.a = a; self.s = s
    def neg(self): return V(self.a, -self.s)

class Prog:
    def __init__(self): self.ops = []; self.pos = 0
    def push(self, f): self.ops.append(f)
    def remaining(self): return len(self.ops) - self.pos
    def run(self, n=None):
        end = len(self.ops) if n is None else min(len(self.ops), self.pos + n)
        while self.pos < end:
            self.ops[self.pos](); self.pos += 1
    def _bin(self, f, a, b):
        c = Cell()
        def t(): c.v = f(a.get(), b.get())
        self.push(t); return c
    def add(self, x, y):
        if x.a is None: return y
        if y.a is None: return x
        if x.s == y.s: return V(self._bin(lambda p, q: p + q, x.a, y.a), x.s)
        if x.s > 0: return V(self._bin(lambda p, q: p - q, x.a, y.a), 1)
        return V(self._bin(lambda p, q: p - q, y.a, x.a), 1)
    def sub(self, x, y): return self.add(x, y.neg())
    def mul(self, x, c):
        if x.a is None or c == 0: return V(None)
        if c == 1: return x
        if c == -1: return x.neg()
        cell = Cell(); k = np.float32(c * x.s); a = x.a
        def t(): cell.v = a.get() * k
        self.push(t); return V(cell, 1)
    def cmul(self, xr, xi, c, s):
        if abs(abs(c) - abs(s)) < 1e-12 and abs(c) > 1e-12:
            if (c > 0) == (s > 0):
                return self.mul(self.sub(xr, xi), c), self.mul(self.add(xr, xi), c)
            else:
                return self.mul(self.add(xr, xi), c), self.mul(self.sub(xi, xr), c)
        return (self.sub(self.mul(xr, c), self.mul(xi, s)), self.add(self.mul(xr, s), self.mul(xi, c)))
    def val(self, x):
        a, s = x.a, x.s
        return (lambda: a.get()) if s > 0 else (lambda: -a.get())
    def spill(self, x, store, load):
        if x.a is None: return x
        a = x.a
        self.push(lambda: store(a.get()))
        return V(Cell(load), x.s)

def _tw(k, n):
    c, s = math.cos(2*math.pi*k/n), -math.sin(2*math.pi*k/n)
    if abs(c) < 1e-12: c = 0.0
    if abs(s) < 1e-12: s = 0.0
    return c, s

def rfft(P, x, spill=None, emit=None):
    n = len(x)
    if n == 1:
        return [x[0]], [V(None)]
    if n == 2:
        return [P.add(x[0], x[1]), P.sub(x[0], x[1])], [V(None), V(None)]
    er, ei = rfft(P, x[0::2])
    if spill is not None:
        er, ei = spill(er, ei)
    orr, oi = rfft(P, x[1::2])
    h = n // 2; q = n // 4
    re = [None]*(h+1); im = [None]*(h+1)
    def done(k):
        if emit is not None: emit(k, re[k], im[k])
    re[0] = P.add(er[0], orr[0]); re[h] = P.sub(er[0], orr[0]); im[0] = V(None); im[h] = V(None)
    done(0); done(h)
    re[q] = er[q]; im[q] = orr[q].neg()
    done(q)
    for k in range(1, q):
        c, s = _tw(k, n)
        tr, ti = P.cmul(orr[k], oi[k], c, s)
        re[k] = P.add(er[k], tr); im[k] = P.add(ei[k], ti)
        done(k)
        re[h-k] = P.sub(er[k], tr); im[h-k] = P.sub(ti, ei[k])
        done(h-k)
    return re, im

def irfft(P, re, im, spill=None, emit=None, _idx=None):
    h = len(re) - 1; n = 2*h
    if _idx is None: _idx = list(range(max(n, 1)))
    if h == 0:
        if emit: emit(_idx[0], re[0])
        return [re[0]]
    if n == 2:
        o = [P.add(re[0], re[1]), P.sub(re[0], re[1])]
        if emit: emit(_idx[0], o[0]); emit(_idx[1], o[1])
        return o
    q = n // 4
    er = [None]*(q+1); ei = [None]*(q+1); orr = [None]*(q+1); oi = [None]*(q+1)
    er[0] = P.add(re[0], re[h]); orr[0] = P.sub(re[0], re[h]); ei[0] = V(None); oi[0] = V(None)
    er[q] = re[q]; orr[q] = im[q].neg(); ei[q] = V(None); oi[q] = V(None)
    for k in range(1, q):
        er[k] = P.add(re[k], re[h-k]); ei[k] = P.sub(im[k], im[h-k])
        tr = P.sub(re[k], re[h-k]); ti = P.add(im[k], im[h-k])
        c, s = _tw(k, n)
        orr[k], oi[k] = P.cmul(tr, ti, c, -s)
    if spill is not None:
        orr, oi = spill(orr, oi)
    xe = irfft(P, er, ei, None, emit, _idx[0::2]); xo = irfft(P, orr, oi, None, emit, _idx[1::2])
    out = [None]*n
    out[0::2] = xe; out[1::2] = xo
    return out

def _fcomb(P, n, k, er, ei, orr, oi):
    h = n // 2; q = n // 4
    if k == 0:
        return [(0, P.add(er, orr), V(None)), (h, P.sub(er, orr), V(None))]
    if k == q:
        return [(q, er, orr.neg())]
    c, s = _tw(k, n)
    tr, ti = P.cmul(orr, oi, c, s)
    return [(k, P.add(er, tr), P.add(ei, ti)), (h-k, P.sub(er, tr), P.sub(ti, ei))]

def rfft64_top(P, F, k):
    E = _fcomb(P, 32, k, F[0][0][k], F[0][1][k], F[2][0][k], F[2][1][k])
    O = _fcomb(P, 32, k, F[1][0][k], F[1][1][k], F[3][0][k], F[3][1][k])
    out = []
    for (kb, er, ei), (kb2, orr, oi) in zip(E, O):
        assert kb == kb2
        out += _fcomb(P, 64, kb, er, ei, orr, oi)
    return out

def _icomb(P, n, k, ar, ai, br, bi):
    q = n // 4
    if k == 0:
        return (P.add(ar, br), V(None)), (P.sub(ar, br), V(None))
    if k == q:
        return (ar, V(None)), (ai.neg(), V(None))
    er = P.add(ar, br); ei = P.sub(ai, bi)
    tr = P.sub(ar, br); ti = P.add(ai, bi)
    c, s = _tw(k, n)
    orr, oi = P.cmul(tr, ti, c, -s)
    return (er, ei), (orr, oi)

def irfft64_top(P, re, im, k):
    def lvl64(kb):
        if kb == 0: return _icomb(P, 64, 0, re[0], None, re[32], None)
        if kb == 16: return _icomb(P, 64, 16, re[16], im[16], None, None)
        return _icomb(P, 64, kb, re[kb], im[kb], re[32-kb], im[32-kb])
    if k == 0:
        E0, O0 = lvl64(0); E16, O16 = lvl64(16)
        F0, F2 = _icomb(P, 32, 0, E0[0], None, E16[0], None)
        F1, F3 = _icomb(P, 32, 0, O0[0], None, O16[0], None)
    elif k == 8:
        E8, O8 = lvl64(8)
        F0, F2 = _icomb(P, 32, 8, E8[0], E8[1], None, None)
        F1, F3 = _icomb(P, 32, 8, O8[0], O8[1], None, None)
    else:
        Ea, Oa = lvl64(k); Eb, Ob = lvl64(16-k)
        F0, F2 = _icomb(P, 32, k, Ea[0], Ea[1], Eb[0], Eb[1])
        F1, F3 = _icomb(P, 32, k, Oa[0], Oa[1], Ob[0], Ob[1])
    return [F0, F1, F2, F3]

def scope(name):
    return contextlib.nullcontext()

H=W=224; C=96; K=7
T=64; HOP=56; NT=H//HOP
KK=K*C
WP=256
BF=jnp.bfloat16; U32=jnp.uint32; F32=jnp.float32
OVL = 1
PU = 8
TOK = 1
LAG = 0

def pack(lo, hi):
    return pltpu.pack_elementwise([lo, hi], packed_dtype=BF)
def unpack(x, i):
    return pltpu.unpack_elementwise(x, index=i, packed_dtype=BF, unpacked_dtype=F32)

def freq_of_slot(q):
    c = q // 2
    if c == 0: return 0 if q == 0 else 16
    return c if q % 2 == 0 else 32 - c

def coef_table():
    tab = np.zeros((16, 8), np.float32)
    for c in range(1, 16):
        th = 2*math.pi*c/T
        tab[c, 0:3] = [math.cos(th*d) for d in (1,2,3)]
        tab[c, 3:6] = [-math.sin(th*d) for d in (1,2,3)]
    return tab

def operm():
    out = []
    for r in range(96):
        m = 2*r if r < 48 else 2*(r-48)+1
        o = 2*m if m < 48 else 2*(m-48)+1
        out.append(o)
    return np.array(out)

def loop(n, f, lo=0):
    def body(i, c):
        f(i); return c
    jax.lax.fori_loop(lo, n, body, 0)

def kern(x_hbm, w_ref, ct_ref, l_ref, o_hbm, x_ref, a_ref, u_ref, xb_ref, xfa_ref, xfb_ref, xfc_ref, xfd_ref,
         yfa_ref, yfb_ref, yfc_ref, yfd_ref, xc_ref, ob_ref, tmp_ref, isem, osem):
    xf_refs = [xfa_ref, xfb_ref, xfc_ref, xfd_ref]
    yf_refs = [yfa_ref, yfb_ref, yfc_ref, yfd_ref]
    chunks = [(216, 8), (0, 56), (56, 56), (112, 56), (168, 48)]
    def in_dma(i):
        s, n = chunks[i]
        return pltpu.make_async_copy(x_hbm.at[0, pl.ds(s, n)], x_ref.at[pl.ds(s, n)], isem.at[i])
    for i in range(5):
        in_dma(i).start()

    with scope("wbase"):
        L = l_ref[...]
        def wT(a):
            r = w_ref[a].reshape(KK, C)
            return jax.lax.dot_general(L, r, (((1,), (1,)), ((), ())), preferred_element_type=F32)
        sc = np.float32(2.0 / T)
        u_ref[0] = wT(3) * sc
        for d in range(1, 4):
            wp = wT(3+d) * sc; wm = wT(3-d) * sc
            u_ref[d] = wp + wm
            u_ref[3+d] = wp - wm
    def put(q, comp, rlo, rhi, v):
        pass
    with scope("wgen"):
        def special(g):
            r = pl.multiple_of(g*8, 8)
            def ld(j): return u_ref[j, pl.ds(r, 8), :], u_ref[j, pl.ds(r+48, 8), :]
            u = [ld(j) for j in range(7)]
            res = []
            for h in range(2):
                w3, s1, s2, s3, t1, t2, t3 = [u[j][h] for j in range(7)]
                e = w3 + s2; o = s1 + s3
                w0 = (e + o) * 0.5; w32 = (e - o) * 0.5
                wr = w3 - s2; wi = t3 - t1
                res.append((jnp.zeros_like(w0), w32, -w0, wr, wi - wr, wr + wi))
            for i in range(6):
                a_ref[i // 3, i % 3, pl.ds(r, 8), :] = pack(res[0][i], res[1][i])
        loop(6, special)
        def gen(c):
            c1, c2, c3, z1, z2, z3 = [ct_ref[c, j] for j in range(6)]
            for g in range(6):
                r = g*8
                res = []
                for h in range(2):
                    w3, s1, s2, s3, t1, t2, t3 = [u_ref[j, r+48*h:r+48*h+8, :] for j in range(7)]
                    er = w3 + s2*c2; orr = s1*c1 + s3*c3
                    ei = t2*z2; oi = t1*z1 + t3*z3
                    wr = er + orr; wi = oi + ei
                    wr2 = er - orr; wi2 = oi - ei
                    res.append((wr, wi - wr, wr + wi, wr2, wi2 - wr2, wr2 + wi2))
                for i in range(6):
                    a_ref[2*c + i // 3, i % 3, r:r+8, :] = pack(res[0][i], res[1][i])
        loop(16, gen, 1)

    def stage_rows(h0, n):
        for k in range(n):
            h = h0 + k
            v = pltpu.bitcast(x_ref[h], U32)
            v0 = v[:, :128]
            v1 = jnp.concatenate([v[:, 128:], jnp.zeros((48, 32), U32)], axis=1)
            lane = jax.lax.broadcasted_iota(jnp.int32, v0.shape, 1)
            e1 = jnp.where(lane >= 122, pltpu.roll(v1, 32, 1), v1)
            xb_ref[h] = jnp.concatenate([v0, e1], axis=1)

    def slot_base(k):
        q = 2*k if k < 16 else (1 if k == 16 else 2*(32-k)+1)
        return 3*q
    def fft_prog(P, t, j, sl):
        r = pl.multiple_of((j // 2) * 8, 8); cc = pl.multiple_of((j % 2) * 128, 128)
        xf_ref = xf_refs[t]
        F = [[None]*4 for _ in range(2)]
        for jj in range(4):
            raw = [Cell(functools.partial(lambda n: xb_ref[(HOP*t - 6 + n) % H, pl.ds(r, 8), pl.ds(cc, 128)], n)) if n < T-2 else None for n in range(jj, T, 4)]
            for h in range(2):
                xs = [V(Cell(functools.partial(lambda c, h: unpack(c.get(), h), c, h))) if c is not None else V(None) for c in raw]
                re, im = rfft(P, xs)
                def sp(v, idx):
                    return P.spill(v, functools.partial(lambda idx, x: tmp_ref.__setitem__((sl, idx), x), idx),
                                   functools.partial(lambda idx: tmp_ref[sl, idx], idx))
                b = (jj*2 + h)*16
                re = [sp(re[k], b + k) for k in range(9)]
                im = [sp(im[k], b + 8 + k) if 0 < k < 8 else im[k] for k in range(9)]
                F[h][jj] = (re, im)
        for k in range(9):
            o0 = rfft64_top(P, F[0], k); o1 = rfft64_top(P, F[1], k)
            for (b, re0, im0), (_, re1, im1) in zip(o0, o1):
                def st(i, lo, hi):
                    flo, fhi = P.val(lo), P.val(hi)
                    P.push(lambda: xf_ref.__setitem__((i, pl.ds(r, 8), pl.ds(cc, 128)), pack(flo(), fhi())))
                if b == 0:
                    st(2, re0, re1); st(0, re0, re1)
                elif b == T//2:
                    st(1, re0, re1)
                else:
                    s0 = P.add(re0, im0); s1 = P.add(re1, im1)
                    q = slot_base(b)
                    st(q, s0, s1); st(q+1, re0, re1); st(q+2, im0, im1)
    def fft_dcol(t, j):
        P = Prog(); fft_prog(P, t, j, 0); P.run()

    def ifft_prog(P, t, j, sl):
        r = pl.multiple_of((j // 2) * 8, 8); cc = pl.multiple_of((j % 2) * 128, 128)
        yf_ref = yf_refs[t]
        Fr = [[[None]*9 for _ in range(4)] for _ in range(2)]; Fi = [[[None]*9 for _ in range(4)] for _ in range(2)]
        for h in range(2):
            ld = lambda i, h=h: V(Cell(lambda: yf_ref[i, pl.ds(r + 48*h, 8), pl.ds(cc, 128)]))
            re = [None]*33; im = [None]*33
            re[0] = ld(0); re[32] = ld(1)
            for k in range(1, 32):
                q = slot_base(k) // 3
                re[k] = ld(2*q); im[k] = ld(2*q+1)
            for k in range(9):
                G = irfft64_top(P, re, im, k)
                for jj in range(4):
                    def sp(v, idx):
                        return P.spill(v, functools.partial(lambda idx, x: tmp_ref.__setitem__((sl, idx), x), idx),
                                       functools.partial(lambda idx: tmp_ref[sl, idx], idx))
                    b = (jj*2 + h)*16
                    Fr[h][jj][k] = sp(G[jj][0], b + k)
                    Fi[h][jj][k] = sp(G[jj][1], b + 8 + k) if 0 < k < 8 else G[jj][1]
        for jj in range(4):
            o0 = irfft(P, Fr[0][jj], Fi[0][jj])
            def emit(m, v, jj=jj, o0=o0):
                n = 4*m + jj
                if 3 <= n < 3 + HOP:
                    flo, fhi = P.val(o0[m]), P.val(v)
                    P.push(lambda: ob_ref.__setitem__((n-3, pl.ds(r, 8), pl.ds(cc, 128)), pack(flo(), fhi())))
            irfft(P, Fr[1][jj], Fi[1][jj], None, emit)
    def ifft_dcol(t, j):
        P = Prog(); ifft_prog(P, t, j, 0); P.run()

    def build_xcol(t, p, slot, only=None):
        for comp in (range(3) if only is None else [only]):
            v = xf_refs[t][3*p+comp]
            v0 = v[:, :128]; v1 = v[:, 128:]
            lane = jax.lax.broadcasted_iota(jnp.int32, v0.shape, 1)
            xc_ref[slot, comp, 0:48] = v
            for b in range(1, K):
                r0 = pltpu.roll(v0, b, 1); r1 = pltpu.roll(v1, b, 1)
                m = lane >= b
                xc_ref[slot, comp, 48*b:48*b+48] = jnp.concatenate([jnp.where(m, r0, r1), jnp.where(m, r1, r0)], axis=1)

    def out_dma(t):
        return pltpu.make_async_copy(x_ref.at[pl.ds(HOP*t, HOP)], o_hbm.at[0, pl.ds(HOP*t, HOP)], osem.at[t])
    def emit_out(t):
        def f(n):
            for k in range(8):
                x_ref[HOP*t + n*8 + k] = pltpu.bitcast(ob_ref[n*8 + k], BF)[:, :W]
        loop(HOP//8, f)
        out_dma(t).start()
    def out_dma_g(g):
        t = NT-1
        return pltpu.make_async_copy(x_ref.at[pl.ds(HOP*t, HOP), pl.ds(16*g, 16)], o_hbm.at[0, pl.ds(HOP*t, HOP), pl.ds(16*g, 16)], osem.at[NT-1+g])

    with scope("stage0"):
        in_dma(0).wait()
        stage_rows(218, 6)
        in_dma(1).wait()
        loop(7, lambda n: stage_rows(n*8, 8))
    with scope("fft0"):
        loop(12, lambda j: fft_dcol(0, j))
    with scope("stage1"):
        in_dma(2).wait()
        loop(7, lambda n: stage_rows(56 + n*8, 8))
    build_xcol(0, 0, 0)
    NI = 32 // PU
    DC = 12 // NI
    for t in range(NT):
        if t == 0: in_dma(3).wait()
        if t == 1: in_dma(4).wait()
        def body(i):
            P = Prog()
            sl = 0
            if OVL and t + 1 < NT:
                for d in range(DC):
                    fft_prog(P, t+1, i*DC + d, sl); sl += 1
            if OVL and t > 0:
                for d in range(DC):
                    ifft_prog(P, t-1, i*DC + d, sl); sl += 1
            nslots = PU * 3
            chunk = -(-len(P.ops) // (nslots - LAG))
            for u in range(PU):
                p = i*PU + u
                pn = p + 1 if u < PU - 1 else jnp.minimum(p+1, 31)
                ps = []
                for comp in range(3):
                    build_xcol(t, pn, (u+1) % 2, comp)
                    xcol = pltpu.bitcast(xc_ref[u % 2, comp], BF)
                    a = pltpu.bitcast(a_ref[p, comp], BF)
                    ps.append(jnp.dot(a, xcol, preferred_element_type=F32))
                    if TOK:
                        tmp_ref[6, i] = ps[-1][0:8, 0:128]
                    P.run(chunk)
                yf_refs[t][2*p] = ps[0] - ps[2]
                yf_refs[t][2*p+1] = ps[0] + ps[1]
                if t < 2 and u < 7:
                    stage_rows(112 + 56*t + 14*i + 2*u, 2)
            P.run()
        with scope("main%d" % t):
            loop(NI, body)
        if not OVL:
            if t + 1 < NT:
                loop(12, lambda j: fft_dcol(t+1, j))
            loop(12, lambda j: ifft_dcol(t, j))
            if t < NT-1: emit_out(t)
        elif t > 0:
            emit_out(t-1)
        if t + 1 < NT:
            build_xcol(t+1, 0, 0)
    with scope("ifft3"):
        def last(g):
            if OVL:
                ifft_dcol(NT-1, 2*g); ifft_dcol(NT-1, 2*g+1)
            r8 = pl.multiple_of(g*8, 8); r16 = pl.multiple_of(g*16, 16)
            for n in range(HOP):
                x_ref[HOP*(NT-1) + n, pl.ds(r16, 16), :] = pltpu.bitcast(ob_ref[n, pl.ds(r8, 8), :], BF)[:, :W]
            out_dma_g(g).start()
        loop(6, last)
    with scope("outwait"):
        for t in range(NT-1):
            out_dma(t).wait()
        for g in range(6):
            out_dma_g(g).wait()

@jax.jit
def pallas_standalone__fft_conv__vision_kernel(x: jax.Array, w: jax.Array):
    xT = x.transpose(0, 1, 3, 2)
    ct = coef_table()
    L = np.zeros((C, C), np.float32); L[np.arange(C), operm()] = 1
    yT = pl.pallas_call(
        kern,
        in_specs=[pl.BlockSpec(memory_space=pl.ANY),
                  pl.BlockSpec(memory_space=pltpu.VMEM),
                  pl.BlockSpec(memory_space=pltpu.SMEM),
                  pl.BlockSpec(memory_space=pltpu.VMEM)],
        out_specs=pl.BlockSpec(memory_space=pl.ANY),
        out_shape=jax.ShapeDtypeStruct((1, H, C, W), BF),
        scratch_shapes=[pltpu.VMEM((H, C, W), BF),
                        pltpu.VMEM((32, 3, 48, KK), U32),
                        pltpu.VMEM((7, C, KK), F32),
                        pltpu.VMEM((H, 48, WP), U32)]
                       + [pltpu.VMEM((96, 48, WP), U32)]*4
                       + [pltpu.VMEM((T, C, WP), F32)]*4
                       + [pltpu.VMEM((2, 3, 48*K, WP), U32),
                        pltpu.VMEM((HOP, 48, WP), U32),
                        pltpu.VMEM((7, 128, 8, 128), F32),
                        pltpu.SemaphoreType.DMA((5,)), pltpu.SemaphoreType.DMA((NT-1+6,))],
        compiler_params=pltpu.CompilerParams(vmem_limit_bytes=120*1024*1024),
    )(xT, w, ct, jnp.asarray(L, BF))
    return yT.transpose(0, 1, 3, 2)
```

```python
import contextlib
import functools
import math

import jax
import jax.numpy as jnp
import numpy as np
import jax.experimental.pallas as pl
import jax.experimental.pallas.tpu as pltpu

class Cell:
    __slots__ = ("v", "fn")
    def __init__(self, fn=None): self.v = None; self.fn = fn
    def get(self):
        if self.v is None: self.v = self.fn()
        return self.v

class V:
    __slots__ = ("s", "a")
    def __init__(self, a, s=1): self.a = a; self.s = s
    def neg(self): return V(self.a, -self.s)

class Prog:
    def __init__(self): self.ops = []; self.pos = 0
    def push(self, f): self.ops.append(f)
    def remaining(self): return len(self.ops) - self.pos
    def run(self, n=None):
        end = len(self.ops) if n is None else min(len(self.ops), self.pos + n)
        while self.pos < end:
            self.ops[self.pos](); self.pos += 1
    def _bin(self, f, a, b):
        c = Cell()
        def t(): c.v = f(a.get(), b.get())
        self.push(t); return c
    def add(self, x, y):
        if x.a is None: return y
        if y.a is None: return x
        if x.s == y.s: return V(self._bin(lambda p, q: p + q, x.a, y.a), x.s)
        if x.s > 0: return V(self._bin(lambda p, q: p - q, x.a, y.a), 1)
        return V(self._bin(lambda p, q: p - q, y.a, x.a), 1)
    def sub(self, x, y): return self.add(x, y.neg())
    def mul(self, x, c):
        if x.a is None or c == 0: return V(None)
        if c == 1: return x
        if c == -1: return x.neg()
        cell = Cell(); k = np.float32(c * x.s); a = x.a
        def t(): cell.v = a.get() * k
        self.push(t); return V(cell, 1)
    def cmul(self, xr, xi, c, s):
        if abs(abs(c) - abs(s)) < 1e-12 and abs(c) > 1e-12:
            if (c > 0) == (s > 0):
                return self.mul(self.sub(xr, xi), c), self.mul(self.add(xr, xi), c)
            else:
                return self.mul(self.add(xr, xi), c), self.mul(self.sub(xi, xr), c)
        return (self.sub(self.mul(xr, c), self.mul(xi, s)), self.add(self.mul(xr, s), self.mul(xi, c)))
    def val(self, x):
        a, s = x.a, x.s
        return (lambda: a.get()) if s > 0 else (lambda: -a.get())
    def spill(self, x, store, load):
        if x.a is None: return x
        a = x.a
        self.push(lambda: store(a.get()))
        return V(Cell(load), x.s)

def _tw(k, n):
    c, s = math.cos(2*math.pi*k/n), -math.sin(2*math.pi*k/n)
    if abs(c) < 1e-12: c = 0.0
    if abs(s) < 1e-12: s = 0.0
    return c, s

def rfft(P, x, spill=None, emit=None):
    n = len(x)
    if n == 1:
        return [x[0]], [V(None)]
    if n == 2:
        return [P.add(x[0], x[1]), P.sub(x[0], x[1])], [V(None), V(None)]
    er, ei = rfft(P, x[0::2])
    if spill is not None:
        er, ei = spill(er, ei)
    orr, oi = rfft(P, x[1::2])
    h = n // 2; q = n // 4
    re = [None]*(h+1); im = [None]*(h+1)
    def done(k):
        if emit is not None: emit(k, re[k], im[k])
    re[0] = P.add(er[0], orr[0]); re[h] = P.sub(er[0], orr[0]); im[0] = V(None); im[h] = V(None)
    done(0); done(h)
    re[q] = er[q]; im[q] = orr[q].neg()
    done(q)
    for k in range(1, q):
        c, s = _tw(k, n)
        tr, ti = P.cmul(orr[k], oi[k], c, s)
        re[k] = P.add(er[k], tr); im[k] = P.add(ei[k], ti)
        done(k)
        re[h-k] = P.sub(er[k], tr); im[h-k] = P.sub(ti, ei[k])
        done(h-k)
    return re, im

def irfft(P, re, im, spill=None, emit=None, _idx=None):
    h = len(re) - 1; n = 2*h
    if _idx is None: _idx = list(range(max(n, 1)))
    if h == 0:
        if emit: emit(_idx[0], re[0])
        return [re[0]]
    if n == 2:
        o = [P.add(re[0], re[1]), P.sub(re[0], re[1])]
        if emit: emit(_idx[0], o[0]); emit(_idx[1], o[1])
        return o
    q = n // 4
    er = [None]*(q+1); ei = [None]*(q+1); orr = [None]*(q+1); oi = [None]*(q+1)
    er[0] = P.add(re[0], re[h]); orr[0] = P.sub(re[0], re[h]); ei[0] = V(None); oi[0] = V(None)
    er[q] = re[q]; orr[q] = im[q].neg(); ei[q] = V(None); oi[q] = V(None)
    for k in range(1, q):
        er[k] = P.add(re[k], re[h-k]); ei[k] = P.sub(im[k], im[h-k])
        tr = P.sub(re[k], re[h-k]); ti = P.add(im[k], im[h-k])
        c, s = _tw(k, n)
        orr[k], oi[k] = P.cmul(tr, ti, c, -s)
    if spill is not None:
        orr, oi = spill(orr, oi)
    xe = irfft(P, er, ei, None, emit, _idx[0::2]); xo = irfft(P, orr, oi, None, emit, _idx[1::2])
    out = [None]*n
    out[0::2] = xe; out[1::2] = xo
    return out

def _fcomb(P, n, k, er, ei, orr, oi):
    h = n // 2; q = n // 4
    if k == 0:
        return [(0, P.add(er, orr), V(None)), (h, P.sub(er, orr), V(None))]
    if k == q:
        return [(q, er, orr.neg())]
    c, s = _tw(k, n)
    tr, ti = P.cmul(orr, oi, c, s)
    return [(k, P.add(er, tr), P.add(ei, ti)), (h-k, P.sub(er, tr), P.sub(ti, ei))]

def rfft64_top(P, F, k):
    E = _fcomb(P, 32, k, F[0][0][k], F[0][1][k], F[2][0][k], F[2][1][k])
    O = _fcomb(P, 32, k, F[1][0][k], F[1][1][k], F[3][0][k], F[3][1][k])
    out = []
    for (kb, er, ei), (kb2, orr, oi) in zip(E, O):
        assert kb == kb2
        out += _fcomb(P, 64, kb, er, ei, orr, oi)
    return out

def _icomb(P, n, k, ar, ai, br, bi):
    q = n // 4
    if k == 0:
        return (P.add(ar, br), V(None)), (P.sub(ar, br), V(None))
    if k == q:
        return (ar, V(None)), (ai.neg(), V(None))
    er = P.add(ar, br); ei = P.sub(ai, bi)
    tr = P.sub(ar, br); ti = P.add(ai, bi)
    c, s = _tw(k, n)
    orr, oi = P.cmul(tr, ti, c, -s)
    return (er, ei), (orr, oi)

def irfft64_top(P, re, im, k):
    def lvl64(kb):
        if kb == 0: return _icomb(P, 64, 0, re[0], None, re[32], None)
        if kb == 16: return _icomb(P, 64, 16, re[16], im[16], None, None)
        return _icomb(P, 64, kb, re[kb], im[kb], re[32-kb], im[32-kb])
    if k == 0:
        E0, O0 = lvl64(0); E16, O16 = lvl64(16)
        F0, F2 = _icomb(P, 32, 0, E0[0], None, E16[0], None)
        F1, F3 = _icomb(P, 32, 0, O0[0], None, O16[0], None)
    elif k == 8:
        E8, O8 = lvl64(8)
        F0, F2 = _icomb(P, 32, 8, E8[0], E8[1], None, None)
        F1, F3 = _icomb(P, 32, 8, O8[0], O8[1], None, None)
    else:
        Ea, Oa = lvl64(k); Eb, Ob = lvl64(16-k)
        F0, F2 = _icomb(P, 32, k, Ea[0], Ea[1], Eb[0], Eb[1])
        F1, F3 = _icomb(P, 32, k, Oa[0], Oa[1], Ob[0], Ob[1])
    return [F0, F1, F2, F3]

R2 = math.sqrt(0.5)
def f4(P, n, k, F):
    q = n // 4; h = n // 2
    if k == 0:
        a = P.add(F[0][0], F[2][0]); b = P.sub(F[0][0], F[2][0]); c = P.add(F[1][0], F[3][0]); d = P.sub(F[1][0], F[3][0])
        return [(0, P.add(a, c), V(None)), (h, P.sub(a, c), V(None)), (q, b, d.neg())]
    if 8*k == n:
        f0, f1, f2, f3 = [F[j][0] for j in range(4)]
        u = P.mul(P.sub(f1, f3), R2); v = P.mul(P.add(f1, f3), R2)
        return [(k, P.add(f0, u), P.add(f2, v).neg()), (q + k, P.sub(f0, u), P.sub(f2, v))]
    T = [F[0]] + [P.cmul(F[j][0], F[j][1], *_tw(j*k, n)) for j in (1, 2, 3)]
    ar, ai = P.add(T[0][0], T[2][0]), P.add(T[0][1], T[2][1]); br, bi = P.sub(T[0][0], T[2][0]), P.sub(T[0][1], T[2][1])
    cr, ci = P.add(T[1][0], T[3][0]), P.add(T[1][1], T[3][1]); dr, di = P.sub(T[1][0], T[3][0]), P.sub(T[1][1], T[3][1])
    return [(k, P.add(ar, cr), P.add(ai, ci)), (h - k, P.sub(ar, cr), P.sub(ci, ai)),
            (q + k, P.add(br, di), P.sub(bi, dr)), (q - k, P.sub(br, di), P.add(bi, dr).neg())]

def i4(P, n, k, re, im):
    q = n // 4; h = n // 2
    Z = V(None)
    if k == 0:
        a = P.add(re[0], re[h]); c = P.sub(re[0], re[h]); b = re[q]; d = im[q].neg()
        return [(P.add(a, b), Z), (P.add(c, d), Z), (P.sub(a, b), Z), (P.sub(c, d), Z)]
    if 8*k == n:
        f0 = P.add(re[k], re[q+k]); u = P.mul(P.sub(re[k], re[q+k]), R2)
        f2 = P.sub(im[q+k], im[k]); v = P.mul(P.add(im[k], im[q+k]), -R2)
        return [(f0, Z), (P.add(u, v), Z), (f2, Z), (P.sub(v, u), Z)]
    ar, ai = P.add(re[k], re[h-k]), P.sub(im[k], im[h-k]); cr, ci = P.sub(re[k], re[h-k]), P.add(im[k], im[h-k])
    br, bi = P.add(re[q+k], re[q-k]), P.sub(im[q+k], im[q-k])
    di = P.sub(re[q+k], re[q-k]); dr = P.add(im[q+k], im[q-k]).neg()
    t0 = (P.add(ar, br), P.add(ai, bi)); t2 = (P.sub(ar, br), P.sub(ai, bi))
    t1 = (P.add(cr, dr), P.add(ci, di)); t3 = (P.sub(cr, dr), P.sub(ci, di))
    out = [t0]
    for j, t in ((1, t1), (2, t2), (3, t3)):
        c, s = _tw(j*k, n)
        out.append(P.cmul(t[0], t[1], c, -s))
    return out

def rfft4(P, x):
    n = len(x)
    if n == 1: return [x[0]], [V(None)]
    F = [rfft4(P, x[j::4]) for j in range(4)]
    re = [None]*(n//2+1); im = [None]*(n//2+1)
    for k in range(n//8 + 1):
        for b, r, i in f4(P, n, k, [(F[j][0][k], F[j][1][k]) for j in range(4)]):
            re[b] = r; im[b] = i
    return re, im

def irfft4(P, re, im, emit=None, _idx=None):
    n = max(2*(len(re)-1), 1)
    if _idx is None: _idx = list(range(n))
    if n == 1:
        if emit: emit(_idx[0], re[0])
        return [re[0]]
    m = n // 8
    Fr = [[None]*(m+1) for _ in range(4)]; Fi = [[None]*(m+1) for _ in range(4)]
    for k in range(m+1):
        G = i4(P, n, k, re, im)
        for j in range(4): Fr[j][k], Fi[j][k] = G[j]
    out = [None]*n
    for j in range(4):
        out[j::4] = irfft4(P, Fr[j], Fi[j], emit, _idx[j::4])
    return out

def scope(name):
    return contextlib.nullcontext()

H=W=224; C=96; K=7
T=64; HOP=56; NT=H//HOP
KK=640
WP=256
BF=jnp.bfloat16; U32=jnp.uint32; F32=jnp.float32
OVL = 1
PU = 8
NOB0 = 1
KSPL = 0
TOK = 1
LAG = 1
EARLY = 1

def pack(lo, hi):
    return pltpu.pack_elementwise([lo, hi], packed_dtype=BF)
def unpack(x, i):
    return pltpu.unpack_elementwise(x, index=i, packed_dtype=BF, unpacked_dtype=F32)

def freq_of_slot(q):
    c = q // 2
    if c == 0: return 0 if q == 0 else 16
    return c if q % 2 == 0 else 32 - c

def coef_table():
    tab = np.zeros((16, 8), np.float32)
    for c in range(1, 16):
        th = 2*math.pi*c/T
        tab[c, 0:3] = [math.cos(th*d) for d in (1,2,3)]
        tab[c, 3:6] = [-math.sin(th*d) for d in (1,2,3)]
    return tab

def operm():
    out = []
    for r in range(96):
        m = 2*r if r < 48 else 2*(r-48)+1
        o = 2*m if m < 48 else 2*(m-48)+1
        out.append(o)
    return np.array(out)

def loop(n, f, lo=0):
    def body(i, c):
        f(i); return c
    jax.lax.fori_loop(lo, n, body, 0)

def kern(x_hbm, w_ref, ct_ref, l_ref, o_hbm, x_ref, a_ref, al_ref, u_ref, xb_ref, xfa_ref, xfb_ref, xfc_ref, xfd_ref,
         yfa_ref, yfb_ref, yfc_ref, yfd_ref, xc_ref, ob_ref, tmp_ref, isem, osem):
    xf_refs = [xfa_ref, xfb_ref, xfc_ref, xfd_ref]
    yf_refs = [yfa_ref, yfb_ref, yfc_ref, yfd_ref]
    chunks = [(216, 8), (0, 56), (56, 56), (112, 56), (168, 48)]
    def in_dma(i):
        s, n = chunks[i]
        return pltpu.make_async_copy(x_hbm.at[0, pl.ds(s, n)], x_ref.at[pl.ds(s, n)], isem.at[i])
    for i in range(5):
        in_dma(i).start()

    with scope("wbase"):
        L = l_ref[...]
        def wT(a):
            r = w_ref[a].reshape(K*C, C)
            r = jnp.concatenate([r, r[KK:]], axis=0)
            return jax.lax.dot_general(L, r, (((1,), (1,)), ((), ())), preferred_element_type=F32)
        sc = np.float32(2.0 / T)
        u_ref[0] = wT(3) * sc
        for d in range(1, 4):
            wp = wT(3+d) * sc; wm = wT(3-d) * sc
            u_ref[d] = wp + wm
            u_ref[3+d] = wp - wm
    with scope("wgen"):
        lo32 = jax.lax.broadcasted_iota(jnp.int32, (8, 64), 1) < 32
        def put(q, r, res):
            for i in range(3):
                a_ref[q, i, pl.ds(r, 8), :] = pack(res[0][i][:, :KK], res[1][i][:, :KK])
            top = [jnp.where(lo32, res[h][3][:, KK:], -res[h][4][:, KK:]) for h in range(2)]
            bot = [jnp.where(lo32, res[h][4][:, KK:], res[h][3][:, KK:]) for h in range(2)]
            al_ref[q, pl.ds(r, 8), :] = pack(top[0], top[1])
            al_ref[q, pl.ds(r + 48, 8), :] = pack(bot[0], bot[1])
        def special(g):
            r = pl.multiple_of(g*8, 8)
            r0 = []; r1 = []
            for h in range(2):
                w3, s1, s2, s3, t1, t2, t3 = [u_ref[j, pl.ds(r + 48*h, 8), :] for j in range(7)]
                e = w3 + s2; o = s1 + s3
                w0 = (e + o) * 0.5; w32 = (e - o) * 0.5
                wr = w3 - s2; wi = t3 - t1
                r0.append((jnp.zeros_like(w0), w32, -w0, w0, w32))
                r1.append((wr, wi - wr, wr + wi, wr, wi))
            for i in range(3):
                a_ref[0, i, pl.ds(r, 8), :] = pack(r0[0][i][:, :KK], r0[1][i][:, :KK])
            top = [jnp.where(lo32, 0.0, r0[h][3][:, KK:]) for h in range(2)]
            bot = [jnp.where(lo32, r0[h][4][:, KK:], 0.0) for h in range(2)]
            al_ref[0, pl.ds(r, 8), :] = pack(top[0], top[1])
            al_ref[0, pl.ds(r + 48, 8), :] = pack(bot[0], bot[1])
            put(1, r, r1)
        loop(6, special)
        def gen(c):
            c1, c2, c3, z1, z2, z3 = [ct_ref[c, j] for j in range(6)]
            for g in range(6):
                r = g*8
                ra = []; rb = []
                for h in range(2):
                    w3, s1, s2, s3, t1, t2, t3 = [u_ref[j, r+48*h:r+48*h+8, :] for j in range(7)]
                    er = w3 + s2*c2; orr = s1*c1 + s3*c3
                    ei = t2*z2; oi = t1*z1 + t3*z3
                    wr = er + orr; wi = oi + ei
                    wr2 = er - orr; wi2 = oi - ei
                    ra.append((wr, wi - wr, wr + wi, wr, wi))
                    rb.append((wr2, wi2 - wr2, wr2 + wi2, wr2, wi2))
                put(2*c, r, ra); put(2*c + 1, r, rb)
        loop(16, gen, 1)

    def stage_rows(h0, n):
        for k in range(n):
            h = h0 + k
            v = pltpu.bitcast(x_ref[h], U32)
            v0 = v[:, :128]
            v1 = jnp.concatenate([v[:, 128:], jnp.zeros((48, 32), U32)], axis=1)
            lane = jax.lax.broadcasted_iota(jnp.int32, v0.shape, 1)
            e1 = jnp.where(lane >= 122, pltpu.roll(v1, 32, 1), v1)
            xb_ref[h] = jnp.concatenate([v0, e1], axis=1)

    def slot_base(k):
        q = 2*k if k < 16 else (1 if k == 16 else 2*(32-k)+1)
        return 3*q
    def fft_prog(P, t, j, sl):
        r = pl.multiple_of((j // 2) * 8, 8); cc = pl.multiple_of((j % 2) * 128, 128)
        xf_ref = xf_refs[t]
        F = [[None]*4 for _ in range(2)]
        for jj in range(4):
            raw = [Cell(functools.partial(lambda n: xb_ref[(HOP*t - 6 + n) % H, pl.ds(r, 8), pl.ds(cc, 128)], n)) if n < T-2 else None for n in range(jj, T, 4)]
            for h in range(2):
                xs = [V(Cell(functools.partial(lambda c, h: unpack(c.get(), h), c, h))) if c is not None else V(None) for c in raw]
                re, im = rfft4(P, xs)
                def sp(v, idx):
                    return P.spill(v, functools.partial(lambda idx, x: tmp_ref.__setitem__((sl, idx), x), idx),
                                   functools.partial(lambda idx: tmp_ref[sl, idx], idx))
                b = (jj*2 + h)*16
                re = [sp(re[k], b + k) for k in range(9)]
                im = [sp(im[k], b + 8 + k) if 0 < k < 8 else im[k] for k in range(9)]
                F[h][jj] = (re, im)
        for k in range(9):
            o0, o1 = [f4(P, T, k, [(F[h][jj][0][k], F[h][jj][1][k]) for jj in range(4)]) for h in range(2)]
            for (b, re0, im0), (_, re1, im1) in zip(o0, o1):
                def st(i, lo, hi):
                    flo, fhi = P.val(lo), P.val(hi)
                    P.push(lambda: xf_ref.__setitem__((i, pl.ds(r, 8), pl.ds(cc, 128)), pack(flo(), fhi())))
                if b == 0:
                    st(2, re0, re1); st(0, re0, re1)
                elif b == T//2:
                    st(1, re0, re1)
                else:
                    s0 = P.add(re0, im0); s1 = P.add(re1, im1)
                    q = slot_base(b)
                    st(q, s0, s1); st(q+1, re0, re1); st(q+2, im0, im1)
    def fft_dcol(t, j):
        P = Prog(); fft_prog(P, t, j, 0); P.run()

    def ifft_prog(P, t, j, sl):
        r = pl.multiple_of((j // 2) * 8, 8); cc = pl.multiple_of((j % 2) * 128, 128)
        yf_ref = yf_refs[t]
        Fr = [[[None]*9 for _ in range(4)] for _ in range(2)]; Fi = [[[None]*9 for _ in range(4)] for _ in range(2)]
        for h in range(2):
            ld = lambda i, h=h: V(Cell(lambda: yf_ref[i, pl.ds(r + 48*h, 8), pl.ds(cc, 128)]))
            re = [None]*33; im = [None]*33
            re[0] = ld(0); re[32] = ld(1)
            for k in range(1, 32):
                q = slot_base(k) // 3
                re[k] = ld(2*q); im[k] = ld(2*q+1)
            for k in range(9):
                G = i4(P, T, k, re, im)
                for jj in range(4):
                    def sp(v, idx):
                        return P.spill(v, functools.partial(lambda idx, x: tmp_ref.__setitem__((sl, idx), x), idx),
                                       functools.partial(lambda idx: tmp_ref[sl, idx], idx))
                    b = (jj*2 + h)*16
                    Fr[h][jj][k] = sp(G[jj][0], b + k)
                    Fi[h][jj][k] = sp(G[jj][1], b + 8 + k) if 0 < k < 8 else G[jj][1]
        for jj in range(4):
            o0 = irfft4(P, Fr[0][jj], Fi[0][jj])
            def emit(m, v, jj=jj, o0=o0):
                n = 4*m + jj
                if 3 <= n < 3 + HOP:
                    flo, fhi = P.val(o0[m]), P.val(v)
                    P.push(lambda: ob_ref.__setitem__((n-3, pl.ds(r, 8), pl.ds(cc, 128)), pack(flo(), fhi())))
            irfft4(P, Fr[1][jj], Fi[1][jj], emit)
    def ifft_dcol(t, j):
        P = Prog(); ifft_prog(P, t, j, 0); P.run()

    def build_xcol(t, p, slot, only=None):
        for comp in (range(3) if only is None else [only]):
            v = xf_refs[t][3*p+comp]
            v0 = v[:, :128]; v1 = v[:, 128:]
            lane = jax.lax.broadcasted_iota(jnp.int32, v0.shape, 1)
            if not NOB0:
                xc_ref[slot, comp, 0:48] = v
            for b in range(1, K):
                r0 = pltpu.roll(v0, b, 1); r1 = pltpu.roll(v1, b, 1)
                m = lane >= b
                e = jnp.concatenate([jnp.where(m, r0, r1), jnp.where(m, r1, r0)], axis=1)
                if comp == 0 and b == K-1:
                    xc_ref[slot, comp, 48*b:48*b+32] = e[:32]
                else:
                    xc_ref[slot, comp, 48*b:48*b+48] = e

    def out_dma(t, hh):
        return pltpu.make_async_copy(x_ref.at[pl.ds(HOP*t, HOP), pl.ds(48*hh, 48)], o_hbm.at[0, pl.ds(HOP*t, HOP), pl.ds(48*hh, 48)], osem.at[2*t + hh])
    def emit_out(t, hh):
        r24 = pl.multiple_of(hh*24, 8); r48 = pl.multiple_of(hh*48, 16)
        def f(n):
            for k in range(14):
                x_ref[HOP*t + n*14 + k, pl.ds(r48, 48), :] = pltpu.bitcast(ob_ref[n*14 + k, pl.ds(r24, 24), :], BF)[:, :W]
        loop(HOP//14, f)
        out_dma(t, hh).start()
    def out_dma3(i):
        t = NT-2
        return pltpu.make_async_copy(x_ref.at[pl.ds(HOP*t, HOP), pl.ds(32*i, 32)], o_hbm.at[0, pl.ds(HOP*t, HOP), pl.ds(32*i, 32)], osem.at[2*(NT-1)+6+i])
    def out_dma_g(g):
        t = NT-1
        return pltpu.make_async_copy(x_ref.at[pl.ds(HOP*t, HOP), pl.ds(16*g, 16)], o_hbm.at[0, pl.ds(HOP*t, HOP), pl.ds(16*g, 16)], osem.at[2*(NT-1)+g])

    with scope("stage0"):
        in_dma(0).wait()
        stage_rows(218, 6)
        in_dma(1).wait()
        loop(7, lambda n: stage_rows(n*8, 8))
    with scope("fft0"):
        loop(12, lambda j: fft_dcol(0, j))
    with scope("stage1"):
        in_dma(2).wait()
        loop(7, lambda n: stage_rows(56 + n*8, 8))
    build_xcol(0, 0, 0)
    NI = 32 // PU
    DC = 12 // NI
    for t in range(NT):
        if t == 0: in_dma(3).wait()
        if t == 1: in_dma(4).wait()
        def body(i):
            P = Prog()
            sl = 0
            if OVL and t + 1 < NT:
                for d in range(DC):
                    fft_prog(P, t+1, i*DC + d, sl); sl += 1
            if OVL and t > 0:
                if EARLY and t == NT-1:
                    for d in range(4):
                        ifft_prog(P, t-1, jnp.minimum(i, 2)*4 + d, sl); sl += 1
                else:
                    for d in range(DC):
                        ifft_prog(P, t-1, i*DC + d, sl); sl += 1
            nslots = PU * 3
            chunk = -(-len(P.ops) // (nslots - LAG))
            for u in range(PU):
                p = i*PU + u
                pn = p + 1 if u < PU - 1 else jnp.minimum(p+1, 31)
                def tok(v):
                    if TOK:
                        tmp_ref[6, i] = v[0:8, 0:128]
                def mm(comp):
                    if NOB0:
                        xr = jnp.concatenate([xf_refs[t][3*p+comp], xc_ref[u % 2, comp, 48:KK//2]], axis=0)
                    else:
                        xr = xc_ref[u % 2, comp, 0:KK//2]
                    xcol = pltpu.bitcast(xr, BF)
                    a = pltpu.bitcast(a_ref[p, comp], BF)
                    if KSPL:
                        acc = None
                        for kt in range(5):
                            d = jnp.dot(a[:, 128*kt:128*kt+128], xcol[128*kt:128*kt+128], preferred_element_type=F32)
                            acc = d if acc is None else acc + d
                        return acc
                    return jnp.dot(a, xcol, preferred_element_type=F32)
                build_xcol(t, pn, (u+1) % 2, 0)
                xl = jnp.concatenate([xc_ref[u % 2, 1, KK//2:], xc_ref[u % 2, 2, KK//2:]], axis=0)
                pl_ = jnp.dot(pltpu.bitcast(al_ref[p], BF), pltpu.bitcast(xl, BF), preferred_element_type=F32)
                p1 = mm(0)
                ur = p1 + pl_[:C]; ui = p1 + pl_[C:]
                tok(p1); P.run(chunk)
                build_xcol(t, pn, (u+1) % 2, 1)
                p2 = mm(1)
                yf_refs[t][2*p+1] = ui + p2
                tok(p2); P.run(chunk)
                build_xcol(t, pn, (u+1) % 2, 2)
                p3 = mm(2)
                yf_refs[t][2*p] = ur - p3
                tok(p3); P.run(chunk)
                if t < 2 and u < 7:
                    stage_rows(112 + 56*t + 14*i + 2*u, 2)
            P.run()
        with scope("main%d" % t):
            if t == 0:
                loop(NI, body)
            elif EARLY and t == NT-1:
                def third(i):
                    body(i)
                    @pl.when(i < 3)
                    def _():
                        r16 = pl.multiple_of(i*16, 8); r32 = pl.multiple_of(i*32, 16)
                        def f(n):
                            for k in range(14):
                                x_ref[HOP*(t-1) + n*14 + k, pl.ds(r32, 32), :] = pltpu.bitcast(ob_ref[n*14 + k, pl.ds(r16, 16), :], BF)[:, :W]
                        loop(HOP//14, f)
                        out_dma3(i).start()
                loop(NI, third)
            else:
                def half(hh):
                    loop(hh*(NI//2) + NI//2, body, hh*(NI//2))
                    emit_out(t-1, hh)
                loop(2, half)
        if t + 1 < NT:
            build_xcol(t+1, 0, 0)
    with scope("ifft3"):
        def last(g):
            ifft_dcol(NT-1, 2*g); ifft_dcol(NT-1, 2*g+1)
            r8 = pl.multiple_of(g*8, 8); r16 = pl.multiple_of(g*16, 16)
            for n in range(HOP):
                x_ref[HOP*(NT-1) + n, pl.ds(r16, 16), :] = pltpu.bitcast(ob_ref[n, pl.ds(r8, 8), :], BF)[:, :W]
            out_dma_g(g).start()
        loop(6, last)
    with scope("outwait"):
        for t in range(NT-2 if EARLY else NT-1):
            for hh in range(2):
                out_dma(t, hh).wait()
        if EARLY:
            for i in range(3):
                out_dma3(i).wait()
        for g in range(6):
            out_dma_g(g).wait()

@jax.jit
def pallas_standalone__fft_conv__vision_kernel(x: jax.Array, w: jax.Array):
    xT = x.transpose(0, 1, 3, 2)
    ct = coef_table()
    L = np.zeros((C, C), np.float32); L[np.arange(C), operm()] = 1
    yT = pl.pallas_call(
        kern,
        in_specs=[pl.BlockSpec(memory_space=pl.ANY),
                  pl.BlockSpec(memory_space=pltpu.VMEM),
                  pl.BlockSpec(memory_space=pltpu.SMEM),
                  pl.BlockSpec(memory_space=pltpu.VMEM)],
        out_specs=pl.BlockSpec(memory_space=pl.ANY),
        out_shape=jax.ShapeDtypeStruct((1, H, C, W), BF),
        scratch_shapes=[pltpu.VMEM((H, C, W), BF),
                        pltpu.VMEM((32, 3, 48, KK), U32),
                        pltpu.VMEM((32, 96, 64), U32),
                        pltpu.VMEM((7, C, KK + 64), F32),
                        pltpu.VMEM((H, 48, WP), U32)]
                       + [pltpu.VMEM((96, 48, WP), U32)]*4
                       + [pltpu.VMEM((T, C, WP), F32)]*4
                       + [pltpu.VMEM((2, 3, 48*K, WP), U32),
                        pltpu.VMEM((HOP, 48, WP), U32),
                        pltpu.VMEM((7, 128, 8, 128), F32),
                        pltpu.SemaphoreType.DMA((5,)), pltpu.SemaphoreType.DMA((2*(NT-1)+9,))],
        compiler_params=pltpu.CompilerParams(vmem_limit_bytes=120*1024*1024),
    )(xT, w, ct, jnp.asarray(L, BF))
    return yT.transpose(0, 1, 3, 2)
```
